```python
import os as _os
_os.environ.setdefault("JAX_PLATFORMS", "cpu")
import jax
import jax.numpy as jnp

def _softmax(x, axis=-1):
    return jax.nn.softmax(x, axis=axis)
def _gelu(x):
    return jax.nn.gelu(x, approximate=True)
def _silu(x):
    return jax.nn.silu(x)
def _sigmoid(x):
    return jax.nn.sigmoid(x)
def _layernorm(x, axis=-1, eps=1e-5):
    m = jnp.mean(x, axis=axis, keepdims=True)
    v = jnp.var(x, axis=axis, keepdims=True)
    return (x - m) / jnp.sqrt(v + eps)
def _scatter_add(tgt, idx, src, axis=0):
    return tgt.at[idx].add(src)
def _segment_sum(src, seg, n):
    return jax.ops.segment_sum(src, seg, n)
class _Rng:
    def __init__(self, key):
        self._k = key
    def _next(self):
        self._k, sub = jax.random.split(self._k)
        return sub
    def normal(self, shape):
        return jax.random.normal(self._next(), shape, dtype=jnp.bfloat16)
    def randint(self, lo, hi, shape):
        return jax.random.randint(self._next(), shape, lo, hi, dtype=jnp.int32)
    def uniform(self, shape, lo=0.0, hi=1.0):
        return jax.random.uniform(self._next(), shape, jnp.bfloat16, lo, hi)
    def permutation(self, n):
        return jax.random.permutation(self._next(), n)


kernel_name = 'concat_heads__grouped_kv_mqa__sliding_block__prompt'

def setup_inputs():
    _rng = _Rng(jax.random.key(int.from_bytes(__import__("os").urandom(4), "little")))
    _w = (lambda a: (lambda t: t.astype(jnp.bfloat16) if jnp.issubdtype(t.dtype, jnp.floating) else t)(jnp.asarray(a)))
    def _A_setup():
        B, S, D, H = 1, 2048, 1024, 32
        Dh = D // H
        return {
            "x": _w((lambda *s: _rng.normal(s) * 0.05)(B, S, D)),
            "wq": _w((lambda *s: _rng.normal(s) * 1.6)(D, H * Dh)),
            "wk": _w((lambda *s: _rng.normal(s) * 1.6)(D, Dh)),
            "wv": _w((lambda *s: _rng.normal(s) * 0.1)(D, Dh)),
            "wo": _w((lambda *s: _rng.normal(s) * 0.1)(H * Dh, D)),
        }
    _A_in = _A_setup()

    def _B_setup():
        B, S, D = 1, 2048, 1024
        return {
            "x": _w((lambda *s: _rng.normal(s) * 0.2)(B, S, D)),
            "wqkv": _w((lambda *s: _rng.normal(s) * 0.2)(D, 3 * D)),
            "wo": _w((lambda *s: _rng.normal(s) * 0.05)(D, D)),
        }
    _B_in = _B_setup()

    return {
        "A_x": _A_in["x"],
        "A_wq": _A_in["wq"],
        "A_wk": _A_in["wk"],
        "A_wv": _A_in["wv"],
        "A_wo": _A_in["wo"],
        "B_x": _B_in["x"],
        "B_wqkv": _B_in["wqkv"],
        "B_wo": _B_in["wo"],
    }

def reference(A_x, A_wq, A_wk, A_wv, A_wo, B_x, B_wqkv, B_wo):
    def _A_ref(x, wq, wk, wv, wo):
        B, S, D = x.shape
        H = 32
        Dh = D // H
        q = (lambda x, *d: x.transpose(*d))((x @ wq).reshape(B, S, H, Dh), 0, 2, 1, 3)
        k = x @ wk
        v = x @ wv
        scores = jnp.einsum("bhqd,bkd->bhqk", q, k) * (Dh ** -0.5)
        p = _softmax(scores, axis=-1)
        o = jnp.einsum("bhqk,bkd->bhqd", p, v)
        return (lambda x, *d: x.transpose(*d))(o, 0, 2, 1, 3).reshape(B, S, H * Dh) @ wo

    def _B_ref(x, wqkv, wo):
        B, S, D = x.shape
        H = 32; Dh = D // H; W = 256
        qkv = (lambda x, *d: x.transpose(*d))((x @ wqkv).reshape(B, S, 3, H, Dh), 2, 0, 3, 1, 4)
        q, k, v = qkv[0], qkv[1], qkv[2]
        scores = jnp.einsum("bhqd,bhkd->bhqk", q, k) * (Dh ** -0.5)
        idx = jnp.arange(S)
        mask = (idx[:, None] - idx[None, :] >= 0) & (idx[:, None] - idx[None, :] < W)
        scores = jnp.where(mask[None, None], scores, -1e9)
        p = _softmax(scores, axis=-1)
        o = jnp.einsum("bhqk,bhkd->bhqd", p, v)
        return (lambda x, *d: x.transpose(*d))(o, 0, 2, 1, 3).reshape(B, S, D) @ wo

    a = _A_ref(A_x, A_wq, A_wk, A_wv, A_wo)
    b = _B_ref(B_x, B_wqkv, B_wo)
    return jnp.concatenate([a, b], axis=-1)
```

```python
import math

import jax
import jax.numpy as jnp
from jax import lax
import jax.experimental.pallas as pl
import jax.experimental.pallas.tpu as pltpu

S = 2048
D = 1024
H = 32
DH = 32
WIN = 256
G = D // 128
KC = 128
NCH = S // KC
NA = 512
UA = 4
NSLOT = NCH * UA
NEG = -1e30
QSCALE = (DH ** -0.5) * math.log2(math.e)

F32 = jnp.float32
BF16 = jnp.bfloat16
NT = (((1,), (1,)), ((), ()))
TN = (((0,), (0,)), ((), ()))


def _kernel(ax_hbm, awq_hbm, awkt_hbm, awvt_hbm, awo_hbm, bx_hbm, bwqkv_hbm, bwo_hbm,
            out_hbm,
            x_ref, wq_ref, wkvt_ref, wqkv_ref, wo_ref,
            qa_ref, ka_ref, vta_ref, qkb_ref, vtb_ref, ot_ref,
            s0_ref, s1_ref, m_ref, sems, osems):
    s_bufs = (s0_ref, s1_ref)

    def copy(i, src, dst):
        return pltpu.make_async_copy(src, dst, sems.at[i])

    half = S // 2
    cp_wkt = copy(0, awkt_hbm, wkvt_ref.at[0:DH])
    cp_wvt = copy(1, awvt_hbm, wkvt_ref.at[DH:2 * DH])
    cp_wq = copy(2, awq_hbm, wq_ref)
    cp_xa = [copy(3 + r, ax_hbm.at[r * half:(r + 1) * half], x_ref.at[0, r * half:(r + 1) * half])
             for r in range(2)]
    cp_xb = copy(5, bx_hbm, x_ref.at[1])
    cp_wqkv = copy(6, bwqkv_hbm, wqkv_ref)
    cp_woa = copy(7, awo_hbm, wo_ref.at[0])
    cp_wob = copy(8, bwo_hbm, wo_ref.at[1])

    cp_wq.start()
    cp_xa[0].start()
    cp_wkt.start()
    cp_wvt.start()
    cp_xa[1].start()

    lane = lax.broadcasted_iota(jnp.int32, (1, 128), 1)

    def proj_a(r, _):
        rows = pl.ds(pl.multiple_of(r * half, half), half)
        x = x_ref[0, rows, :]
        y = jnp.dot(x, wq_ref[...], preferred_element_type=F32)
        for g in range(G):
            qa_ref[g, rows, :] = (y[:, g * 128:(g + 1) * 128] * QSCALE).astype(BF16)
        kvt = lax.dot_general(wkvt_ref[...], x, NT, preferred_element_type=F32)
        vta_ref[:, rows] = kvt[DH:2 * DH, :].astype(BF16)
        kt = kvt[0:DH, :]
        k4 = jnp.concatenate([kt, kt, kt, kt], axis=0).T
        for j in range(4):
            mine = (lane >= j * DH) & (lane < (j + 1) * DH)
            ka_ref[j, rows, :] = jnp.where(mine, k4, 0.0).astype(BF16)
        return _

    cp_wq.wait()
    cp_wkt.wait()
    cp_wvt.wait()
    cp_xa[0].wait()
    cp_xb.start()
    cp_wqkv.start()
    cp_woa.start()
    cp_wob.start()
    cp_xa[1].wait()
    lax.fori_loop(0, 2, proj_a, 0)

    def col_max(acc, s):
        mm = jnp.max(s.reshape(s.shape[0] // 8, 8, s.shape[1]), axis=0)
        return mm if acc is None else jnp.maximum(acc, mm)

    def col_sum(acc, p):
        ll = jnp.sum(p.reshape(p.shape[0] // 8, 8, p.shape[1]), axis=0)
        return ll if acc is None else acc + ll

    n_qb = S // NA
    n_units_a = H * n_qb
    G2A = 2

    def a_unit(u):
        return u // n_qb, u % n_qb

    def a_stage(u_next, u_cur, nxt, cur):
        for uu in range(UA):
            if u_next is not None:
                h1, qb1 = a_unit(u_next + uu)
                w = qa_ref[h1 // 4, pl.ds(pl.multiple_of(qb1 * NA, NA), NA), :]
                kj = h1 % 4
            if u_cur is not None:
                h2, qb2 = a_unit(u_cur + uu)
                m = m_ref[cur, uu]
            m8 = None
            npc = NA // (128 * G2A)
            l8 = [None] * npc
            acc = [None] * npc
            for j in range(NCH):
                slot = uu * NCH + j
                keys = slice(j * KC, (j + 1) * KC)
                if u_cur is not None:
                    for c in range(npc):
                        cs = slice(c * G2A * 128, (c + 1) * G2A * 128)
                        p = jnp.exp2(s_bufs[cur][slot, :, cs] - m[:, cs])
                        oo = jnp.dot(vta_ref[:, keys], p.astype(BF16), preferred_element_type=F32)
                        acc[c] = oo if acc[c] is None else acc[c] + oo
                        l8[c] = col_sum(l8[c], p)
                if u_next is not None:
                    s = lax.dot_general(ka_ref[kj, keys, :], w, NT, preferred_element_type=F32)
                    s_bufs[nxt][slot] = s
                    m8 = col_max(m8, s)
            if u_next is not None:
                m_ref[nxt, uu] = jnp.max(m8, axis=0, keepdims=True)
            if u_cur is not None:
                for c in range(npc):
                    inv = 1.0 / jnp.sum(l8[c], axis=0, keepdims=True)
                    ot_ref[0, pl.ds(pl.multiple_of(h2 * DH, DH), DH),
                           pl.ds(pl.multiple_of(qb2 * NA + c * G2A * 128, 128), G2A * 128)] = (
                               acc[c] * inv).astype(BF16)

    n_stage_a = n_units_a // UA
    a_stage(0, None, 0, None)

    def a_body(i, _):
        @pl.when(i % 2 == 0)
        def _even():
            a_stage((i + 1) * UA, i * UA, 1, 0)

        @pl.when(i % 2 == 1)
        def _odd():
            a_stage((i + 1) * UA, i * UA, 0, 1)
        return _

    lax.fori_loop(0, n_stage_a - 1, a_body, 0)
    a_stage(None, (n_stage_a - 1) * UA, None, (n_stage_a - 1) % 2)

    cp_xb.wait()
    cp_wqkv.wait()

    def proj_qk_b(t, _):
        which = t // 2
        rows = pl.ds(pl.multiple_of((t % 2) * half, half), half)
        w = wqkv_ref[:, pl.ds(pl.multiple_of(which * D, D), D)]
        y = jnp.dot(x_ref[1, rows, :], w, preferred_element_type=F32)
        scale = jnp.where(which == 0, QSCALE, 1.0).astype(F32)
        for g in range(G):
            qkb_ref[which, g, rows, :] = (y[:, g * 128:(g + 1) * 128] * scale).astype(BF16)
        return _

    lax.fori_loop(0, 4, proj_qk_b, 0)

    def proj_v_b(r, _):
        rows = pl.ds(pl.multiple_of(r * half, half), half)
        y = jnp.dot(x_ref[1, rows, :], wqkv_ref[:, 2 * D:3 * D], preferred_element_type=F32)
        vtb_ref[:, rows] = y.astype(BF16).T
        return _

    lax.fori_loop(0, 2, proj_v_b, 0)

    row_i = lax.broadcasted_iota(jnp.int32, (KC, 128), 0)
    col_i = lax.broadcasted_iota(jnp.int32, (KC, 128), 1)
    lane_u = lax.broadcasted_iota(jnp.int32, (KC // 2, 128), 1)

    def b_chunks(qt_static):
        ch = [(-2, "old"), (-1, None), (0, "diag")]
        if qt_static is None:
            return ch
        return [c for c in ch if qt_static + c[0] >= 0]

    def b_stage(qt_next, qt_cur, nxt, cur, next_static=None, cur_static=None):
        ch_next = b_chunks(next_static) if qt_next is not None else []
        ch_cur = b_chunks(cur_static) if qt_cur is not None else []
        for g in range(G):
            if qt_next is not None:
                q = qkb_ref[0, g, pl.ds(pl.multiple_of(qt_next * 128, 128), 128), :]
                qi = pltpu.bitcast(q, jnp.uint32)
                w = jnp.concatenate(
                    [pltpu.bitcast(
                        jnp.where((lane_u >= j * DH) & (lane_u < (j + 1) * DH), qi, jnp.uint32(0)),
                        BF16) for j in range(4)], axis=0)
            if qt_cur is not None:
                m = m_ref[cur, g]
            m8 = None
            l8 = [None] * 4
            acc = [None] * 4
            for c in range(max(len(ch_next), len(ch_cur))):
                slot = g * 3 + c
                if c < len(ch_cur):
                    kt0 = pl.multiple_of((qt_cur + ch_cur[c][0]) * KC, KC)
                    for j in range(4):
                        cs = slice(j * 128, (j + 1) * 128)
                        p = jnp.exp2(s_bufs[cur][slot, :, cs] - m[:, cs])
                        vt = vtb_ref[(4 * g + j) * DH:(4 * g + j + 1) * DH, pl.ds(kt0, KC)]
                        oo = jnp.dot(vt, p.astype(BF16), preferred_element_type=F32)
                        acc[j] = oo if acc[j] is None else acc[j] + oo
                        l8[j] = col_sum(l8[j], p)
                if c < len(ch_next):
                    off, kind = ch_next[c]
                    kt0 = pl.multiple_of((qt_next + off) * KC, KC)
                    s = lax.dot_general(qkb_ref[1, g, pl.ds(kt0, KC), :], w, NT,
                                        preferred_element_type=F32)
                    if kind is not None:
                        keep = (row_i > col_i) if kind == "old" else (row_i <= col_i)
                        s = jnp.concatenate(
                            [jnp.where(keep, s[:, j * 128:(j + 1) * 128], NEG) for j in range(4)],
                            axis=1)
                    s_bufs[nxt][slot] = s
                    m8 = col_max(m8, s)
            if qt_next is not None:
                m_ref[nxt, g] = jnp.max(m8, axis=0, keepdims=True)
            if qt_cur is not None:
                for j in range(4):
                    inv = 1.0 / jnp.sum(l8[j], axis=0, keepdims=True)
                    ot_ref[1, (4 * g + j) * DH:(4 * g + j + 1) * DH,
                           pl.ds(pl.multiple_of(qt_cur * 128, 128), 128)] = (acc[j] * inv).astype(BF16)

    b_stage(0, None, 0, None, next_static=0)
    b_stage(1, 0, 1, 0, next_static=1, cur_static=0)
    b_stage(2, 1, 0, 1, next_static=2, cur_static=1)

    def b_body(qt, _):
        @pl.when(qt % 2 == 0)
        def _even():
            b_stage(qt + 1, qt, 1, 0)

        @pl.when(qt % 2 == 1)
        def _odd():
            b_stage(qt + 1, qt, 0, 1)
        return _

    lax.fori_loop(2, NCH - 1, b_body, 0)
    b_stage(None, NCH - 1, None, (NCH - 1) % 2)

    cp_woa.wait()
    cp_wob.wait()

    def out_copy(t):
        br = t // 2
        rows = pl.ds(pl.multiple_of((t % 2) * half, half), half)
        return pltpu.make_async_copy(
            x_ref.at[br, rows, :],
            out_hbm.at[rows, pl.ds(pl.multiple_of(br * D, D), D)],
            osems.at[t])

    def proj_out(t, _):
        br = t // 2
        rows = pl.ds(pl.multiple_of((t % 2) * half, half), half)
        y = lax.dot_general(ot_ref[br, :, rows], wo_ref[br], TN, preferred_element_type=F32)
        x_ref[br, rows, :] = y.astype(BF16)
        out_copy(t).start()
        return _

    lax.fori_loop(0, 4, proj_out, 0)
    for t in range(4):
        out_copy(t).wait()


@jax.jit
def pallas_concat_heads__grouped_kv_mqa__sliding_block__prompt_kernel(
    A_x: jax.Array,
    A_wq: jax.Array,
    A_wk: jax.Array,
    A_wv: jax.Array,
    A_wo: jax.Array,
    B_x: jax.Array,
    B_wqkv: jax.Array,
    B_wo: jax.Array,
):
    assert A_x.shape == (1, S, D) and B_x.shape == (1, S, D)
    assert A_wq.shape == (D, H * DH) and A_wk.shape == (D, DH) and A_wv.shape == (D, DH)
    assert A_wo.shape == (H * DH, D) and B_wqkv.shape == (D, 3 * D) and B_wo.shape == (D, D)

    any_spec = pl.BlockSpec(memory_space=pl.ANY)
    out = pl.pallas_call(
        _kernel,
        out_shape=jax.ShapeDtypeStruct((S, 2 * D), BF16),
        in_specs=[any_spec] * 8,
        out_specs=any_spec,
        scratch_shapes=[
            pltpu.VMEM((2, S, D), BF16),
            pltpu.VMEM((D, D), BF16),
            pltpu.VMEM((2 * DH, D), BF16),
            pltpu.VMEM((D, 3 * D), BF16),
            pltpu.VMEM((2, D, D), BF16),
            pltpu.VMEM((G, S, 128), BF16),
            pltpu.VMEM((4, S, 128), BF16),
            pltpu.VMEM((DH, S), BF16),
            pltpu.VMEM((2, G, S, 128), BF16),
            pltpu.VMEM((D, S), BF16),
            pltpu.VMEM((2, D, S), BF16),
            pltpu.VMEM((NSLOT, KC, NA), F32),
            pltpu.VMEM((NSLOT, KC, NA), F32),
            pltpu.VMEM((2, G, 1, NA), F32),
            pltpu.SemaphoreType.DMA((9,)),
            pltpu.SemaphoreType.DMA((4,)),
        ],
        compiler_params=pltpu.CompilerParams(vmem_limit_bytes=112 * 1024 * 1024),
    )(A_x.reshape(S, D), A_wq, A_wk.T, A_wv.T, A_wo, B_x.reshape(S, D), B_wqkv, B_wo)
    return out.reshape(1, S, 2 * D)
```

```python
import functools
import math

import jax
import jax.numpy as jnp
from jax import lax
import jax.experimental.pallas as pl
import jax.experimental.pallas.tpu as pltpu

S = 2048
D = 1024
H = 32
DH = 32
WIN = 256
G = D // 128
KC = 128
NCH = S // KC
NA = 512
UA = 8
NSLOT = NCH * UA
MA = 512
MP = 1024
B_STAGES = (7, 6, 3)
WQ_CUTS = (0, 256, 512, D)
TAIL_CUTS = (0, 512, 896, D)
NEG = -1e30
QSCALE = (DH ** -0.5) * math.log2(math.e)

F32 = jnp.float32
BF16 = jnp.bfloat16
U32 = jnp.uint32
NT = (((1,), (1,)), ((), ()))
TN = (((0,), (0,)), ((), ()))

assert WIN == 2 * KC and NA == 4 * KC and S // NA == 4 and S // MP == 2
assert sum(B_STAGES) == NCH and 2 * G * max(B_STAGES) <= NSLOT


def _mo(i, n):
    return i if isinstance(i, int) else pl.multiple_of(i, n)


def _run(fs):
    for f in fs:
        f()


def _col_max(acc, s):
    mm = jnp.max(s.reshape(s.shape[0] // 8, 8, s.shape[1]), axis=0)
    return mm if acc is None else jnp.maximum(acc, mm)


def _col_sum(acc, p):
    ll = jnp.sum(p.reshape(p.shape[0] // 8, 8, p.shape[1]), axis=0)
    return ll if acc is None else acc + ll


def _weave(steps, reads, pieces):
    total = sum(c for c, _, _ in pieces)
    done = spent = 0
    for t, f in enumerate(steps):
        f()
        while (done < len(pieces) and pieces[done][1] <= reads[t]
               and (spent + pieces[done][0]) * len(steps) <= (t + 1) * total + 1e-6):
            spent += pieces[done][0]
            pieces[done][2]()
            done += 1
    for _, _, f in pieces[done:]:
        f()


def _kernel(ax_hbm, awq_hbm, awkt_hbm, awvt_hbm, awo_hbm, bx_hbm, bwqkv_hbm, bwo_hbm,
            out_hbm,
            x_ref, wq_ref, wkvt_ref, wqkv_ref, wo_ref,
            qa_ref, ka_ref, vta_ref, qkb_ref, vtb_ref, ot_ref,
            s_ref, ma_ref, mb_ref, tri_ref, one_ref, sems, osems):

    def copy(i, src, dst):
        return pltpu.make_async_copy(src, dst, sems.at[i])

    n_ra = S // MA
    cp_wkt = copy(0, awkt_hbm, wkvt_ref.at[0:DH])
    cp_wvt = copy(1, awvt_hbm, wkvt_ref.at[DH:2 * DH])
    cp_xb = copy(2, bx_hbm, x_ref.at[1])
    cp_wqkv = copy(3, bwqkv_hbm, wqkv_ref)
    cp_woa = copy(4, awo_hbm, wo_ref.at[0])
    cp_wob = copy(5, bwo_hbm, wo_ref.at[1])

    def cp_xa(r):
        rows = pl.ds(_mo(r * MA, MA), MA)
        return copy(6 + r, ax_hbm.at[rows], x_ref.at[0, rows])

    def cp_wq(c):
        lo, hi = WQ_CUTS[c], WQ_CUTS[c + 1]
        return copy(6 + n_ra + c, awq_hbm.at[:, lo:hi], wq_ref.at[:, lo:hi])

    cp_xa(0).start()
    cp_wkt.start()
    cp_wvt.start()
    cp_wq(0).start()

    QB = KC // 2
    NBLK = WIN // QB
    lane = lax.broadcasted_iota(jnp.int32, (1, 128), 1)
    r64 = lax.broadcasted_iota(jnp.int32, (QB, 128), 0)
    l64 = lax.broadcasted_iota(jnp.int32, (QB, 128), 1)
    keep_old = r64 > jnp.bitwise_and(l64, QB - 1)
    low = l64 < QB
    lane8 = lax.broadcasted_iota(jnp.int32, (8, 128), 1)
    lane_masks = [jnp.where((lane8 >= j * DH) & (lane8 < (j + 1) * DH), -1, 0).astype(U32)
                  for j in range(4)]
    tri_ref[...] = jnp.where(keep_old, 1.0, 0.0)
    one_ref[0] = 1

    def region(fn):
        pl.when(one_ref[0] == 1)(fn)

    def proj_a_kv(r):
        rows = pl.ds(_mo(r * MA, MA), MA)
        kvt = lax.dot_general(wkvt_ref[...], x_ref[0, rows, :], NT,
                              preferred_element_type=F32)
        vta_ref[:, rows] = kvt[DH:2 * DH, :].astype(BF16)
        kt = kvt[0:DH, :]
        k4 = jnp.concatenate([kt, kt, kt, kt], axis=0).T
        for j in range(4):
            mine = (lane >= j * DH) & (lane < (j + 1) * DH)
            ka_ref[j, rows, :] = jnp.where(mine, k4, 0.0).astype(BF16)

    def proj_a_q(r, lo, hi):
        rows = pl.ds(_mo(r * MA, MA), MA)
        y = jnp.dot(x_ref[0, rows, :], wq_ref[:, lo:hi], preferred_element_type=F32)
        for g in range(lo // 128, hi // 128):
            v = (y[:, g * 128 - lo:(g + 1) * 128 - lo] * QSCALE).astype(BF16)
            qa_ref[g, pl.ds(_mo(r * (MA // 2), MA // 2), MA // 2), :] = pltpu.bitcast(v, U32)

    def proj_a(r, carry):
        cp_xa(r).wait()
        proj_a_kv(r)
        proj_a_q(r, 0, D)
        return carry

    cp_wkt.wait()
    cp_wvt.wait()
    cp_xa(0).wait()
    cp_wq(0).wait()
    cp_wq(1).start()
    cp_wq(2).start()
    proj_a_kv(0)
    proj_a_q(0, WQ_CUTS[0], WQ_CUTS[1])
    cp_wq(1).wait()
    cp_xa(1).start()
    proj_a_q(0, WQ_CUTS[1], WQ_CUTS[2])
    cp_wq(2).wait()
    for r in range(2, n_ra):
        cp_xa(r).start()
    proj_a_q(0, WQ_CUTS[2], WQ_CUTS[3])
    cp_xb.start()
    cp_wqkv.start()
    lax.fori_loop(1, n_ra, proj_a, 0)
    cp_woa.start()
    cp_wob.start()

    n_qb = S // NA
    TA = 2

    def a_unit(u):
        if isinstance(u, int):
            return u // n_qb, u % n_qb
        return lax.shift_right_logical(u, 2), jnp.bitwise_and(u, n_qb - 1)

    def a_steps(u_next, u_cur):
        n_pc = NA // (128 * TA)
        st1, st2 = {}, {}

        def qk(uu, j, c):
            d = st1.setdefault(uu, dict(m8=[None] * n_pc))
            if "w" not in d:
                h1, qb1 = a_unit(u_next + uu)
                g1 = h1 // 4 if isinstance(h1, int) else lax.shift_right_logical(h1, 2)
                d["kj"] = h1 % 4 if isinstance(h1, int) else jnp.bitwise_and(h1, 3)
                d["w"] = pltpu.bitcast(
                    qa_ref[g1, pl.ds(_mo(qb1 * (NA // 2), NA // 2), NA // 2), :], BF16)
            cs = slice(c * TA * 128, (c + 1) * TA * 128)
            s = lax.dot_general(ka_ref[d["kj"], j * KC:(j + 1) * KC, :], d["w"][cs, :], NT,
                                preferred_element_type=F32)
            s_ref[uu * NCH + j, :, cs] = s
            d["m8"][c] = _col_max(d["m8"][c], s)
            if j == NCH - 1 and c == n_pc - 1:
                ma_ref[uu] = jnp.concatenate(
                    [jnp.max(v, axis=0, keepdims=True) for v in d["m8"]], axis=1)

        def pv(uu, j, c):
            d = st2.setdefault(uu, dict(l8=[None] * n_pc, acc=[None] * n_pc))
            if "m" not in d:
                d["m"] = ma_ref[uu]
            cs = slice(c * TA * 128, (c + 1) * TA * 128)
            p = jnp.exp2(s_ref[uu * NCH + j, :, cs] - d["m"][:, cs])
            oo = jnp.dot(vta_ref[:, j * KC:(j + 1) * KC], p.astype(BF16), preferred_element_type=F32)
            d["acc"][c] = oo if d["acc"][c] is None else d["acc"][c] + oo
            d["l8"][c] = _col_sum(d["l8"][c], p)
            if j == NCH - 1:
                h2, qb2 = a_unit(u_cur + uu)
                inv = 1.0 / jnp.sum(d["l8"][c], axis=0, keepdims=True)
                ot_ref[0, pl.ds(_mo(h2 * DH, DH), DH),
                       pl.ds(_mo(qb2 * NA + c * TA * 128, 128), TA * 128)] = (
                           d["acc"][c] * inv).astype(BF16)

        lag = 1 if (u_next is not None and u_cur is not None) else 0

        def step(t):
            do_qk = u_next is not None and 0 <= t - lag < UA * NCH
            do_pv = u_cur is not None and t < UA * NCH
            if do_pv:
                pv(*divmod(t, NCH), 0)
            if do_qk:
                qk(*divmod(t - lag, NCH), 0)
                qk(*divmod(t - lag, NCH), 1)
            if do_pv:
                pv(*divmod(t, NCH), 1)

        return [functools.partial(step, t) for t in range(UA * NCH + lag)]

    n_stage_a = H * n_qb // UA
    _run(a_steps(0, None))

    def proj_v_b(r, carry):
        rows = pl.ds(_mo(r * MP, MP), MP)
        y = jnp.dot(x_ref[1, rows, :], wqkv_ref[:, 2 * D:3 * D], preferred_element_type=F32)
        vtb_ref[:, rows] = y.astype(BF16).T
        return carry

    def proj_qk_b(t, carry):
        which = lax.shift_right_logical(t, 1)
        rows = pl.ds(_mo(jnp.bitwise_and(t, 1) * MP, MP), MP)
        scale = jnp.where(which == 0, QSCALE, 1.0).astype(F32)
        w = wqkv_ref[:, pl.ds(_mo(which * D, D), D)]
        y = jnp.dot(x_ref[1, rows, :], w, preferred_element_type=F32)
        for g in range(G):
            qkb_ref[which, g, rows, :] = (y[:, g * 128:(g + 1) * 128] * scale).astype(BF16)
        return carry

    cp_xb.wait()
    cp_wqkv.wait()
    lax.fori_loop(0, S // MP, proj_v_b, 0)
    lax.fori_loop(0, 2 * (S // MP), proj_qk_b, 0)

    def a_body(i, carry):
        _run(a_steps((i + 1) * UA, i * UA))
        return carry

    lax.fori_loop(0, n_stage_a - 1, a_body, 0)

    def keys(qt, blk):
        k0 = qt * KC - WIN + blk * QB
        return slice(k0, k0 + QB)

    def have(qt, blk):
        return qt * KC - WIN + blk * QB >= 0

    def second_slot(qt):
        return have(qt, NBLK)

    def b_qk(qt, g, u, groups):
        st = {"m8": None}

        def weights(f):
            if ("w", f) not in st:
                qi = pltpu.bitcast(qkb_ref[0, g, qt * KC + f * QB:qt * KC + (f + 1) * QB, :], U32)
                st["w", f] = jnp.concatenate(
                    [pltpu.bitcast(jnp.bitwise_and(qi, jnp.concatenate(
                        [lane_masks[2 * pair + (lh + f) % 2]] * (QB // 16), axis=0)), BF16)
                     for pair in range(2) for lh in range(2)], axis=0)
            return st["w", f]

        def scores(f, blks):
            got = [b for b in blks if have(qt, f + b)]
            out = {}
            if got:
                lhs = jnp.concatenate([qkb_ref[1, g, keys(qt, f + b), :] for b in got], axis=0)
                s = lax.dot_general(lhs, weights(f), NT, preferred_element_type=F32)
                out = {b: s[i * QB:(i + 1) * QB] for i, b in enumerate(got)}
            return [out.get(b) for b in blks]

        def both(fn, *xs):
            return jnp.concatenate([fn(*[x[:, c * 128:(c + 1) * 128] for x in xs]) for c in range(2)],
                                   axis=1)

        def piece(blks, last):
            live = [b for b in blks if b < 2 or second_slot(qt)]

            def f():
                if live:
                    halves = []
                    for hf in range(2):
                        kb = [k for b in live for k in ((0, NBLK) if b == 0 else (b,))]
                        sc = dict(zip(kb, scores(hf, kb)))
                        out = []
                        for b in live:
                            if b == 0 and sc[0] is None:
                                out.append(both(lambda y: jnp.where(keep_old, NEG, y), sc[NBLK]))
                            elif b == 0:
                                out.append(both(lambda x, y: jnp.where(keep_old, x, y),
                                                sc[0], sc[NBLK]))
                            else:
                                out.append(jnp.full((QB, 256), NEG, F32) if sc[b] is None else sc[b])
                        halves.append(out)
                    for i, b in enumerate(live):
                        s = jnp.concatenate([halves[hf][i][:, pair * 128:(pair + 1) * 128]
                                             for pair in range(2) for hf in range(2)], axis=1)
                        s_ref[2 * u + b // 2, (b % 2) * QB:(b % 2 + 1) * QB, :] = s
                        st["m8"] = _col_max(st["m8"], s)
                if last:
                    mb_ref[u] = jnp.max(st["m8"], axis=0, keepdims=True)

            cost = max(sum(have(qt, hf + k) for b in live for k in ((0, NBLK) if b == 0 else (b,)))
                       for hf in range(2)) / 2
            return cost, 2 * u + max(blks) // 2, f

        return [piece(blks, i == len(groups) - 1) for i, blks in enumerate(groups)]

    def b_pv(qt, g, u, rg):
        st = {}
        lowr = low[0:rg]

        def prob(j, b, r):
            if "m" not in st:
                st["m"] = mb_ref[u]
            cs = slice(j * 128, (j + 1) * 128)
            r0 = (b % 2) * QB + r
            p = jnp.exp2(s_ref[2 * u + b // 2, r0:r0 + rg, cs] - st["m"][:, cs])
            st["l", j] = _col_sum(st.get(("l", j)), p)
            return p

        def acc(h, t, parts):
            rows = slice((4 * g + h) * DH, (4 * g + h + 1) * DH)
            oo = jnp.dot(vtb_ref[rows, (qt - 2 + t) * KC:(qt - 1 + t) * KC],
                         jnp.concatenate(parts, axis=0).astype(BF16), preferred_element_type=F32)
            st["o", h] = oo if ("o", h) not in st else st["o", h] + oo

        def pick(i, a, b):
            return jnp.where(lowr, a, b) if i == 0 else jnp.where(lowr, b, a)

        def outer(pair):
            ja, jb = 2 * pair, 2 * pair + 1
            zero = jnp.zeros((rg, 128), F32)
            blk = {(i, b): [] for i in range(2) for b in (0, 1, 4, 5)}
            for r in range(0, QB, rg):
                oda, odb = prob(ja, 0, r), prob(jb, 0, r)
                tri = tri_ref[r:r + rg, :]
                old_a, old_b = oda * tri, odb * tri
                dg_a, dg_b = oda - old_a, odb - old_b
                m1a = prob(ja, 1, r)
                m3b = prob(jb, 3, r) if second_slot(qt) else zero
                for i in range(2):
                    if qt >= 2:
                        blk[i, 0].append(pick(i, old_a, zero))
                        blk[i, 1].append(pick(i, m1a, old_b))
                    blk[i, 4].append(pick(i, dg_a, m3b))
                    blk[i, 5].append(pick(i, zero, dg_b))
            for i in range(2):
                if qt >= 2:
                    acc(2 * pair + i, 0, blk[i, 0] + blk[i, 1])
                acc(2 * pair + i, 2, blk[i, 4] + blk[i, 5])

        def inner(pair):
            ja, jb = 2 * pair, 2 * pair + 1
            blk = {(i, b): [] for i in range(2) for b in (2, 3)}
            for r in range(0, QB, rg):
                m1b = prob(jb, 1, r)
                if second_slot(qt):
                    m2a, m3a, m2b = prob(ja, 2, r), prob(ja, 3, r), prob(jb, 2, r)
                    for i in range(2):
                        blk[i, 2].append(pick(i, m2a, m1b))
                        blk[i, 3].append(pick(i, m3a, m2b))
            if qt >= 1:
                for i in range(2):
                    acc(2 * pair + i, 1, blk[i, 2] + blk[i, 3])
            ia = 1.0 / jnp.sum(st["l", ja], axis=0, keepdims=True)
            ib = 1.0 / jnp.sum(st["l", jb], axis=0, keepdims=True)
            for i in range(2):
                h = 2 * pair + i
                inv = jnp.where(low[0:1], ia, ib) if i == 0 else jnp.where(low[0:1], ib, ia)
                o = st["o", h] * inv
                if i:
                    o = pltpu.roll(o, QB, 1)
                ot_ref[1, (4 * g + h) * DH:(4 * g + h + 1) * DH,
                       qt * KC:(qt + 1) * KC] = o.astype(BF16)

        return [(functools.partial(outer, 0), 2 * u - 1), (functools.partial(inner, 0), 2 * u - 1),
                (functools.partial(outer, 1), 2 * u - 1), (functools.partial(inner, 1), 2 * u + 1)]

    def b_units(k):
        q0 = sum(B_STAGES[:k])
        return [(u, qt, g) for u, (qt, g) in enumerate(
            (qt, g) for g in range(G) for qt in range(q0, q0 + B_STAGES[k]))]

    def b_qk_stage(k, groups):
        return [p for u, qt, g in b_units(k) for p in b_qk(qt, g, u, groups)]

    def b_pv_stage(k, rg):
        sr = [x for u, qt, g in b_units(k) for x in b_pv(qt, g, u, rg)]
        return [f for f, _ in sr], [r for _, r in sr]

    def out_rows(t, r0=0, nr=MP):
        br = t // 2 if isinstance(t, int) else lax.shift_right_logical(t, 1)
        rb = t % 2 if isinstance(t, int) else jnp.bitwise_and(t, 1)
        return br, pl.ds(_mo(rb * MP + r0, nr), nr)

    def out_copy(t, c0=0, nc=D, sem=None):
        br, rows = out_rows(t)
        return pltpu.make_async_copy(x_ref.at[br, rows, c0:c0 + nc],
                                     out_hbm.at[rows, pl.ds(_mo(br * D + c0, 128), nc)],
                                     osems.at[t if sem is None else sem])

    def out_piece(t, r0, nr, c0, nc):
        br, rows = out_rows(t, r0, nr)
        y = lax.dot_general(ot_ref[br, :, rows], wo_ref[br, :, c0:c0 + nc], TN,
                            preferred_element_type=F32)
        x_ref[br, rows, c0:c0 + nc] = y.astype(BF16)

    def proj_out(t, carry):
        out_piece(t, 0, MP, 0, D)
        out_copy(t).start()
        return carry

    fine, coarse = ((0,), (1,), (2, 3)), ((0, 1), (2, 3))

    def a_drain():
        drain = a_steps(None, (n_stage_a - 1) * UA)
        _weave(drain, list(range(len(drain))), b_qk_stage(0, fine))

    def b_drain():
        steps, _ = b_pv_stage(2, 32)
        _weave(steps, [0] * len(steps),
               [(1, 0, functools.partial(out_piece, 0, r, 256, c, 128))
                for r in range(0, MP, 256) for c in range(0, D, 128)])
        out_copy(0).start()

    cp_woa.wait()
    cp_wob.wait()
    region(a_drain)
    region(lambda: _weave(*b_pv_stage(0, 16), b_qk_stage(1, fine)))
    region(lambda: _weave(*b_pv_stage(1, 32), b_qk_stage(2, coarse)))
    lax.fori_loop(1, 3, proj_out, 0)
    region(b_drain)

    def last(i):
        lo, hi = TAIL_CUTS[i], TAIL_CUTS[i + 1]
        out_piece(3, 0, MP, lo, hi - lo)
        out_copy(3, lo, hi - lo, 3 + i).start()

    for i in range(len(TAIL_CUTS) - 1):
        region(functools.partial(last, i))
    for t in range(3):
        out_copy(t).wait()
    for i in range(len(TAIL_CUTS) - 1):
        out_copy(3, TAIL_CUTS[i], TAIL_CUTS[i + 1] - TAIL_CUTS[i], 3 + i).wait()


@jax.jit
def pallas_concat_heads__grouped_kv_mqa__sliding_block__prompt_kernel(
    A_x: jax.Array,
    A_wq: jax.Array,
    A_wk: jax.Array,
    A_wv: jax.Array,
    A_wo: jax.Array,
    B_x: jax.Array,
    B_wqkv: jax.Array,
    B_wo: jax.Array,
):
    assert A_x.shape == (1, S, D) and B_x.shape == (1, S, D)
    assert A_wq.shape == (D, H * DH) and A_wk.shape == (D, DH) and A_wv.shape == (D, DH)
    assert A_wo.shape == (H * DH, D) and B_wqkv.shape == (D, 3 * D) and B_wo.shape == (D, D)

    any_spec = pl.BlockSpec(memory_space=pl.ANY)
    out = pl.pallas_call(
        _kernel,
        out_shape=jax.ShapeDtypeStruct((S, 2 * D), BF16),
        in_specs=[any_spec] * 8,
        out_specs=any_spec,
        scratch_shapes=[
            pltpu.VMEM((2, S, D), BF16),
            pltpu.VMEM((D, D), BF16),
            pltpu.VMEM((2 * DH, D), BF16),
            pltpu.VMEM((D, 3 * D), BF16),
            pltpu.VMEM((2, D, D), BF16),
            pltpu.VMEM((G, S // 2, 128), U32),
            pltpu.VMEM((4, S, 128), BF16),
            pltpu.VMEM((DH, S), BF16),
            pltpu.VMEM((2, G, S, 128), BF16),
            pltpu.VMEM((D, S), BF16),
            pltpu.VMEM((2, D, S), BF16),
            pltpu.VMEM((NSLOT, KC, NA), F32),
            pltpu.VMEM((UA, 1, NA), F32),
            pltpu.VMEM((G * max(B_STAGES), 1, NA), F32),
            pltpu.VMEM((KC // 2, 128), F32),
            pltpu.SMEM((1,), jnp.int32),
            pltpu.SemaphoreType.DMA((6 + S // MA + len(WQ_CUTS) - 1,)),
            pltpu.SemaphoreType.DMA((3 + len(TAIL_CUTS) - 1,)),
        ],
        compiler_params=pltpu.CompilerParams(vmem_limit_bytes=100 * 1024 * 1024),
    )(A_x.reshape(S, D), A_wq, A_wk.T, A_wv.T, A_wo, B_x.reshape(S, D), B_wqkv, B_wo)
    return out.reshape(1, S, 2 * D)
```
